```python
import jax
import jax.numpy as jnp

def _softmax(x, axis=-1):
    return jax.nn.softmax(x, axis=axis)
def _gelu(x):
    return jax.nn.gelu(x, approximate=True)
def _silu(x):
    return jax.nn.silu(x)
def _sigmoid(x):
    return jax.nn.sigmoid(x)
def _layernorm(x, axis=-1, eps=1e-5):
    m = jnp.mean(x, axis=axis, keepdims=True)
    v = jnp.var(x, axis=axis, keepdims=True)
    return (x - m) / jnp.sqrt(v + eps)
def _scatter_add(tgt, idx, src, axis=0):
    return tgt.at[idx].add(src)
def _segment_sum(src, seg, n):
    return jax.ops.segment_sum(src, seg, n)
class _Rng:
    def __init__(self, key):
        self._k = key
    def _next(self):
        self._k, sub = jax.random.split(self._k)
        return sub
    def normal(self, shape):
        return jax.random.normal(self._next(), shape, dtype=jnp.bfloat16)
    def randint(self, lo, hi, shape):
        return jax.random.randint(self._next(), shape, lo, hi, dtype=jnp.int32)
    def uniform(self, shape, lo=0.0, hi=1.0):
        return jax.random.uniform(self._next(), shape, jnp.bfloat16, lo, hi)
    def permutation(self, n):
        return jax.random.permutation(self._next(), n)


kernel_name = 'gated_mix__sliding_local_dilated__glu_gated_reglu__prompt'

def setup_inputs():
    _rng = _Rng(jax.random.key(int.from_bytes(__import__("os").urandom(4), "little")))
    _w = (lambda a: (lambda t: t.astype(jnp.bfloat16) if jnp.issubdtype(t.dtype, jnp.floating) else t)(jnp.asarray(a)))
    def _A_setup():
        B, S, D = 1, 2048, 1024
        return {
            "x": _w((lambda *s: _rng.normal(s) * 0.05)(B, S, D)),
            "wqkv": _w((lambda *s: _rng.normal(s) * 0.05)(D, 3 * D)),
            "wo": _w((lambda *s: _rng.normal(s) * 0.05)(D, D)),
        }
    _A_in = _A_setup()

    def _B_setup():
        B, S, D, F = 1, 2048, 1024, 3584
        return {
            "x": _w((lambda *s: _rng.normal(s) * 0.05)(B, S, D)),
            "W_gate": _w((lambda *s: _rng.normal(s) * 0.05)(D, F) * (2.0 / D) ** 0.5),
            "W_up": _w((lambda *s: _rng.normal(s) * 0.05)(D, F) * (2.0 / D) ** 0.5),
            "W_down": _w((lambda *s: _rng.normal(s) * 0.05)(F, D) * (1.0 / F) ** 0.5),
        }
    _B_in = _B_setup()

    return {
        "A_x": _A_in["x"],
        "A_wqkv": _A_in["wqkv"],
        "A_wo": _A_in["wo"],
        "B_x": _B_in["x"],
        "B_W_gate": _B_in["W_gate"],
        "B_W_up": _B_in["W_up"],
        "B_W_down": _B_in["W_down"],
        "gate_w": _w((lambda *s: _rng.normal(s) * 0.05)(1024)),
    }

def reference(A_x, A_wqkv, A_wo, B_x, B_W_gate, B_W_up, B_W_down, gate_w):
    def _A_ref(x, wqkv, wo):
        B, S, D = x.shape
        H = 32; Dh = D // H
        W, dil = 8, 2
        qkv = (lambda x, *d: x.transpose(*d))((x @ wqkv).reshape(B, S, 3, H, Dh), 2, 0, 3, 1, 4)
        q, k, v = qkv[0], qkv[1], qkv[2]
        scale = Dh ** -0.5
        pos = jnp.arange(S)
        off = jnp.arange(W) * dil
        idx = pos[:, None] - off[None, :]
        mask = idx >= 0
        idx_c = jnp.where(mask, idx, 0).reshape(-1)
        kg = k[:, :, idx_c, :].reshape(B, H, S, W, Dh)
        vg = v[:, :, idx_c, :].reshape(B, H, S, W, Dh)
        logits = jnp.einsum("bhsd,bhswd->bhsw", q, kg) * scale
        logits = jnp.where(mask[None, None, :, :], logits, -1e9)
        attn = _softmax(logits, axis=-1)
        o = jnp.einsum("bhsw,bhswd->bhsd", attn, vg)
        return (lambda x, *d: x.transpose(*d))(o, 0, 2, 1, 3).reshape(B, S, D) @ wo

    def _B_ref(x, W_gate, W_up, W_down):
        gate = jnp.einsum("bsd,df->bsf", x, W_gate)
        up = jnp.einsum("bsd,df->bsf", x, W_up)
        gate = gate * (lambda x, dt: x.astype(dt))(gate > 0, gate.dtype)
        h = gate * up
        return jnp.einsum("bsf,fd->bsd", h, W_down)

    x = A_x
    g = _sigmoid((x * gate_w).sum(-1, keepdims=True))
    a = _A_ref(x, A_wqkv, A_wo)
    b = _B_ref(x, B_W_gate, B_W_up, B_W_down)
    return g * a + (1 - g) * b
```

```python
import functools

import jax
import jax.numpy as jnp
import jax.experimental.pallas as pl
import jax.experimental.pallas.tpu as pltpu

_H = 32
_W = 8
_DIL = 2
_HALO = 16

_T = 512
_FC = 512


def _swap_col_lane_bits(cols):
    lane = jax.lax.broadcasted_iota(jnp.int32, cols[0].shape, 1)
    cols = list(cols)
    for b in range(3):
        s = 4 << b
        hi = (lane & s) != 0
        new = list(cols)
        for a in range(8):
            if a & (1 << b):
                continue
            A, B = cols[a], cols[a | (1 << b)]
            new[a] = jnp.where(hi, pltpu.roll(B, s, 1), A)
            new[a | (1 << b)] = jnp.where(hi, B, pltpu.roll(A, 128 - s, 1))
        cols = new
    return cols


def _kernel(x_ref, gw_ref, wqkv_hbm, wo_hbm, wg_hbm, wu_hbm, wd_hbm, o_ref,
            wqkv_raw, wqkv_ref, wo_ref, wg_ref, wu_ref, wd_ref, k_scr, v_scr, sems,
            *, T, FC, D, F):
    i = pl.program_id(0)
    nf = F // FC

    def cp_g(j):
        return pltpu.make_async_copy(wg_hbm.at[:, pl.ds(j * FC, FC)], wg_ref.at[j], sems.at[3 * j])

    def cp_u(j):
        return pltpu.make_async_copy(wu_hbm.at[:, pl.ds(j * FC, FC)], wu_ref.at[j], sems.at[3 * j + 1])

    def cp_d(j):
        return pltpu.make_async_copy(wd_hbm.at[pl.ds(j * FC, FC), :], wd_ref.at[j], sems.at[3 * j + 2])

    cp_qkv = pltpu.make_async_copy(wqkv_hbm, wqkv_raw, sems.at[3 * nf])
    cp_o = pltpu.make_async_copy(wo_hbm, wo_ref, sems.at[3 * nf + 1])

    @pl.when(i == 0)
    def _():
        for j in range(nf):
            cp_g(j).start()
            cp_u(j).start()
            cp_d(j).start()
        cp_qkv.start()
        cp_o.start()
        k_scr[:, pl.ds(0, _HALO), :] = jnp.zeros((8, _HALO, 128), jnp.float32)
        v_scr[:, pl.ds(0, _HALO), :] = jnp.zeros((8, _HALO, 128), jnp.float32)

    x = x_ref[...]

    acc = None
    for j in range(nf):
        @pl.when(i == 0)
        def _():
            cp_g(j).wait()
            cp_u(j).wait()
            cp_d(j).wait()
        gate = jnp.dot(x, wg_ref[j], preferred_element_type=jnp.float32)
        up = jnp.dot(x, wu_ref[j], preferred_element_type=jnp.float32)
        h = (jnp.where(gate > 0, gate, 0.0) * up).astype(jnp.bfloat16)
        d = jnp.dot(h, wd_ref[j], preferred_element_type=jnp.float32)
        acc = d if acc is None else acc + d

    @pl.when(i == 0)
    def _():
        cp_qkv.wait()
        cp_o.wait()
        RB = 64
        def body(r, c):
            r0 = pl.multiple_of(r * RB, RB)
            for m in range(3):
                cols = [pltpu.bitcast(wqkv_raw[pl.ds(r0, RB), pl.ds(m * D + g * 128, 128)], jnp.uint32)
                        for g in range(8)]
                cols = _swap_col_lane_bits(cols)
                for g in range(8):
                    wqkv_ref[pl.ds(r0, RB), pl.ds(m * D + g * 128, 128)] = pltpu.bitcast(cols[g], jnp.bfloat16)
            return c
        jax.lax.fori_loop(0, D // RB, body, 0)

    q = jnp.dot(x, wqkv_ref[:, pl.ds(0, D)], preferred_element_type=jnp.float32)
    k = jnp.dot(x, wqkv_ref[:, pl.ds(D, D)], preferred_element_type=jnp.float32)
    v = jnp.dot(x, wqkv_ref[:, pl.ds(2 * D, D)], preferred_element_type=jnp.float32)
    for c in range(8):
        k_scr[c, pl.ds(_HALO, T), :] = k[:, c * 128:(c + 1) * 128]
        v_scr[c, pl.ds(_HALO, T), :] = v[:, c * 128:(c + 1) * 128]

    scale = (D // _H) ** -0.5
    lane_i = jax.lax.broadcasted_iota(jnp.int32, (128, 128), 0)
    lane_j = jax.lax.broadcasted_iota(jnp.int32, (128, 128), 1)
    E = jnp.where((lane_i >> 2) == (lane_j >> 2), 1.0, 0.0).astype(jnp.bfloat16)
    row = i * T + jax.lax.broadcasted_iota(jnp.int32, (T, 128), 0)
    logits = []
    for w in range(_W):
        part = None
        for c in range(8):
            t = q[:, c * 128:(c + 1) * 128] * k_scr[c, pl.ds(_HALO - _DIL * w, T), :]
            part = t if part is None else part + t
        l = jnp.dot(part.astype(jnp.bfloat16), E, preferred_element_type=jnp.float32) * scale
        if w > 0:
            l = jnp.where(row >= _DIL * w, l, -1e9)
        logits.append(l)
    mx = logits[0]
    for w in range(1, _W):
        mx = jnp.maximum(mx, logits[w])
    ps = [jnp.exp(l - mx) for l in logits]
    den = ps[0]
    for w in range(1, _W):
        den = den + ps[w]
    inv = 1.0 / den
    ps = [p * inv for p in ps]
    ocols = []
    for c in range(8):
        oc = None
        for w in range(_W):
            t = ps[w] * v_scr[c, pl.ds(_HALO - _DIL * w, T), :]
            oc = t if oc is None else oc + t
        ocols.append(pltpu.bitcast(oc.astype(jnp.bfloat16), jnp.uint32))
    ocols = _swap_col_lane_bits(ocols)
    o = jnp.concatenate([pltpu.bitcast(oc, jnp.bfloat16) for oc in ocols], axis=1)
    a = jnp.dot(o, wo_ref[...], preferred_element_type=jnp.float32)

    k_scr[:, pl.ds(0, _HALO), :] = k_scr[:, pl.ds(T, _HALO), :]
    v_scr[:, pl.ds(0, _HALO), :] = v_scr[:, pl.ds(T, _HALO), :]

    gl = jnp.sum(x.astype(jnp.float32) * gw_ref[...].astype(jnp.float32), axis=-1, keepdims=True)
    g = jax.nn.sigmoid(gl)
    o_ref[...] = (g * a + (1.0 - g) * acc).astype(o_ref.dtype)


@jax.jit
def pallas_gated_mix__sliding_local_dilated__glu_gated_reglu__prompt_kernel(
    A_x: jax.Array,
    A_wqkv: jax.Array,
    A_wo: jax.Array,
    B_x: jax.Array,
    B_W_gate: jax.Array,
    B_W_up: jax.Array,
    B_W_down: jax.Array,
    gate_w: jax.Array,
):
    del B_x
    B, S, D = A_x.shape
    F = B_W_gate.shape[1]
    T, FC = _T, _FC
    nf = F // FC
    x2 = A_x.reshape(B * S, D)
    gw2 = gate_w.reshape(1, D)
    any_spec = pl.BlockSpec(memory_space=pl.ANY)
    out = pl.pallas_call(
        functools.partial(_kernel, T=T, FC=FC, D=D, F=F),
        grid=(S // T,),
        in_specs=[
            pl.BlockSpec((T, D), lambda i: (i, 0)),
            pl.BlockSpec((1, D), lambda i: (0, 0)),
            any_spec, any_spec, any_spec, any_spec, any_spec,
        ],
        out_specs=pl.BlockSpec((T, D), lambda i: (i, 0)),
        out_shape=jax.ShapeDtypeStruct((B * S, D), A_x.dtype),
        scratch_shapes=[
            pltpu.VMEM((D, 3 * D), jnp.bfloat16),
            pltpu.VMEM((D, 3 * D), jnp.bfloat16),
            pltpu.VMEM((D, D), jnp.bfloat16),
            pltpu.VMEM((nf, D, FC), jnp.bfloat16),
            pltpu.VMEM((nf, D, FC), jnp.bfloat16),
            pltpu.VMEM((nf, FC, D), jnp.bfloat16),
            pltpu.VMEM((8, T + _HALO, 128), jnp.float32),
            pltpu.VMEM((8, T + _HALO, 128), jnp.float32),
            pltpu.SemaphoreType.DMA((3 * nf + 2,)),
        ],
        compiler_params=pltpu.CompilerParams(
            dimension_semantics=("arbitrary",),
            vmem_limit_bytes=100 * 1024 * 1024,
        ),
    )(x2, gw2, A_wqkv, A_wo, B_W_gate, B_W_up, B_W_down)
    return out.reshape(B, S, D)
```

```python
import functools

import jax
import jax.numpy as jnp
import jax.experimental.pallas as pl
import jax.experimental.pallas.tpu as pltpu

_H = 32
_W = 8
_DIL = 2
_HALO = 16

_T = 512
_FC = 896


def _swap_col_lane_bits(cols):
    lane = jax.lax.broadcasted_iota(jnp.int32, cols[0].shape, 1)
    cols = list(cols)
    for b in range(3):
        s = 4 << b
        hi = (lane & s) != 0
        new = list(cols)
        for a in range(8):
            if a & (1 << b):
                continue
            A, B = cols[a], cols[a | (1 << b)]
            new[a] = jnp.where(hi, pltpu.roll(B, s, 1), A)
            new[a | (1 << b)] = jnp.where(hi, B, pltpu.roll(A, 128 - s, 1))
        cols = new
    return cols


def _kernel(x_ref, gw_ref, wqkv_hbm, wo_hbm, wg_hbm, wu_hbm, wd_hbm, o_ref,
            raw_ref, wqkv_ref, wo_ref, wg_ref, wu_ref, wd_ref, qkv_scr, halo_scr, att_scr, acc_ref, sems,
            *, T, FC, D, F):
    i = pl.program_id(0)
    nf = F // FC
    R = T // nf

    def cp_g(j):
        return pltpu.make_async_copy(wg_hbm.at[:, pl.ds(j * FC, FC)], wg_ref.at[j], sems.at[0, j])

    def cp_u(j):
        return pltpu.make_async_copy(wu_hbm.at[:, pl.ds(j * FC, FC)], wu_ref.at[j], sems.at[1, j])

    def cp_d(j):
        return pltpu.make_async_copy(wd_hbm.at[pl.ds(j * FC, FC), :], wd_ref.at[j], sems.at[2, j])

    def cp_qkv(m):
        return pltpu.make_async_copy(wqkv_hbm.at[:, pl.ds(m * D, D)], raw_ref.at[m], sems.at[3, m])

    cp_o = pltpu.make_async_copy(wo_hbm, wo_ref, sems.at[3, 3])

    @pl.when(i == 0)
    def _():
        cp_qkv(0).start()
        cp_qkv(1).start()
        halo_scr[...] = jnp.zeros(halo_scr.shape, jnp.float32)

    def qkv_body(m, carry):
        @pl.when(i == 0)
        def _():
            cp_qkv(m).wait()

            @pl.when(m == 0)
            def _():
                cp_qkv(2).start()

            @pl.when(m == 1)
            def _():
                cp_g(0).start()
                cp_u(0).start()

            @pl.when(m == 2)
            def _():
                cp_d(0).start()

            RB = 128
            def body(r, c):
                r0 = pl.multiple_of(r * RB, RB)
                cols = [pltpu.bitcast(raw_ref[m, pl.ds(r0, RB), pl.ds(g * 128, 128)], jnp.uint32)
                        for g in range(8)]
                cols = _swap_col_lane_bits(cols)
                for g in range(8):
                    wqkv_ref[m, pl.ds(r0, RB), pl.ds(g * 128, 128)] = pltpu.bitcast(cols[g], jnp.bfloat16)
                return c
            jax.lax.fori_loop(0, D // RB, body, 0)

        y = jnp.dot(x_ref[...], wqkv_ref[m], preferred_element_type=jnp.float32)
        for c in range(8):
            yc = y[:, c * 128:(c + 1) * 128]
            for s in range(nf):
                if s == 0:
                    qkv_scr[m, s, c, pl.ds(0, _HALO), :] = halo_scr[m, c]
                    qkv_scr[m, s, c, pl.ds(_HALO, R), :] = yc[0:R]
                else:
                    qkv_scr[m, s, c] = yc[s * R - _HALO:(s + 1) * R]
            halo_scr[m, c] = yc[T - _HALO:T]
        return carry
    jax.lax.fori_loop(0, 3, qkv_body, 0)

    scale = (D // _H) ** -0.5
    li = jax.lax.broadcasted_iota(jnp.int32, (128, 128), 0)
    lj = jax.lax.broadcasted_iota(jnp.int32, (128, 128), 1)
    E = jnp.where((li >> 2) == (lj >> 2), 1.0, 0.0).astype(jnp.bfloat16)

    def attn_strip(s):
        row = i * T + s * R + jax.lax.broadcasted_iota(jnp.int32, (R, 128), 0)
        q = [qkv_scr[0, s, c, pl.ds(_HALO, R), :] for c in range(8)]
        logits = []
        for w in range(_W):
            part = None
            for c in range(8):
                t = q[c] * qkv_scr[1, s, c, pl.ds(_HALO - _DIL * w, R), :]
                part = t if part is None else part + t
            l = jnp.dot(part.astype(jnp.bfloat16), E, preferred_element_type=jnp.float32) * scale
            if w > 0:
                l = jnp.where(row >= _DIL * w, l, -1e9)
            logits.append(l)
        mx = logits[0]
        for w in range(1, _W):
            mx = jnp.maximum(mx, logits[w])
        ps = [jnp.exp(l - mx) for l in logits]
        den = ps[0]
        for w in range(1, _W):
            den = den + ps[w]
        inv = 1.0 / den
        ps = [p * inv for p in ps]
        ocols = []
        for c in range(8):
            oc = None
            for w in range(_W):
                t = ps[w] * qkv_scr[2, s, c, pl.ds(_HALO - _DIL * w, R), :]
                oc = t if oc is None else oc + t
            ocols.append(pltpu.bitcast(oc.astype(jnp.bfloat16), jnp.uint32))
        ocols = _swap_col_lane_bits(ocols)
        for c in range(8):
            att_scr[s, :, pl.ds(c * 128, 128)] = pltpu.bitcast(ocols[c], jnp.bfloat16)

    def ffn_body(j, carry):
        @pl.when(i == 0)
        def _():
            cp_g(j).wait()
            cp_u(j).wait()
            cp_d(j).wait()

            @pl.when(j + 1 < nf)
            def _():
                cp_g(j + 1).start()
                cp_u(j + 1).start()
                cp_d(j + 1).start()

            @pl.when(j + 2 == nf)
            def _():
                cp_o.start()

        @pl.when(j == 0)
        def _():
            acc_ref[...] = jnp.zeros(acc_ref.shape, jnp.float32)

        attn_strip(j)
        x = x_ref[...]
        gate = jnp.dot(x, wg_ref[j], preferred_element_type=jnp.float32)
        up = jnp.dot(x, wu_ref[j], preferred_element_type=jnp.float32)
        h = (jnp.where(gate > 0, gate, 0.0) * up).astype(jnp.bfloat16)
        acc_ref[...] += jnp.dot(h, wd_ref[j], preferred_element_type=jnp.float32)
        return carry
    jax.lax.fori_loop(0, nf, ffn_body, 0)

    @pl.when(i == 0)
    def _():
        cp_o.wait()

    a = jnp.dot(att_scr[...].reshape(T, D), wo_ref[...], preferred_element_type=jnp.float32)
    gl = jnp.sum(x_ref[...].astype(jnp.float32) * gw_ref[...].astype(jnp.float32), axis=-1, keepdims=True)
    g = jax.nn.sigmoid(gl)
    o_ref[...] = (g * a + (1.0 - g) * acc_ref[...]).astype(o_ref.dtype)


@jax.jit
def pallas_gated_mix__sliding_local_dilated__glu_gated_reglu__prompt_kernel(
    A_x: jax.Array,
    A_wqkv: jax.Array,
    A_wo: jax.Array,
    B_x: jax.Array,
    B_W_gate: jax.Array,
    B_W_up: jax.Array,
    B_W_down: jax.Array,
    gate_w: jax.Array,
):
    del B_x
    B, S, D = A_x.shape
    F = B_W_gate.shape[1]
    T, FC = _T, _FC
    nf = F // FC
    x2 = A_x.reshape(B * S, D)
    gw2 = gate_w.reshape(1, D)
    any_spec = pl.BlockSpec(memory_space=pl.ANY)
    out = pl.pallas_call(
        functools.partial(_kernel, T=T, FC=FC, D=D, F=F),
        grid=(S // T,),
        in_specs=[
            pl.BlockSpec((T, D), lambda i: (i, 0)),
            pl.BlockSpec((1, D), lambda i: (0, 0)),
            any_spec, any_spec, any_spec, any_spec, any_spec,
        ],
        out_specs=pl.BlockSpec((T, D), lambda i: (i, 0)),
        out_shape=jax.ShapeDtypeStruct((B * S, D), A_x.dtype),
        scratch_shapes=[
            pltpu.VMEM((3, D, D), jnp.bfloat16),
            pltpu.VMEM((3, D, D), jnp.bfloat16),
            pltpu.VMEM((D, D), jnp.bfloat16),
            pltpu.VMEM((nf, D, FC), jnp.bfloat16),
            pltpu.VMEM((nf, D, FC), jnp.bfloat16),
            pltpu.VMEM((nf, FC, D), jnp.bfloat16),
            pltpu.VMEM((3, nf, 8, T // nf + _HALO, 128), jnp.float32),
            pltpu.VMEM((3, 8, _HALO, 128), jnp.float32),
            pltpu.VMEM((nf, T // nf, D), jnp.bfloat16),
            pltpu.VMEM((T, D), jnp.float32),
            pltpu.SemaphoreType.DMA((4, max(nf, 4))),
        ],
        compiler_params=pltpu.CompilerParams(
            dimension_semantics=("arbitrary",),
            vmem_limit_bytes=100 * 1024 * 1024,
        ),
    )(x2, gw2, A_wqkv, A_wo, B_W_gate, B_W_up, B_W_down)
    return out.reshape(B, S, D)
```

```python
import functools

import jax
import jax.numpy as jnp
import jax.experimental.pallas as pl
import jax.experimental.pallas.tpu as pltpu

_H = 32
_W = 8
_DIL = 2
_HALO = 16

_T = 512
_FC = 896


def _swap_col_lane_bits(cols):
    lane = jax.lax.broadcasted_iota(jnp.int32, cols[0].shape, 1)
    cols = list(cols)
    for b in range(3):
        s = 4 << b
        hi = (lane & s) != 0
        new = list(cols)
        for a in range(8):
            if a & (1 << b):
                continue
            A, B = cols[a], cols[a | (1 << b)]
            new[a] = jnp.where(hi, pltpu.roll(B, s, 1), A)
            new[a | (1 << b)] = jnp.where(hi, B, pltpu.roll(A, 128 - s, 1))
        cols = new
    return cols


def _kernel(x_ref, gw_ref, wqkv_hbm, wo_hbm, wg_hbm, wu_hbm, wd_hbm, o_ref,
            wqkv_ref, wo_ref, wg_ref, wu_ref, wd_ref, qkv_scr, halo_scr, att_scr, acc_ref, sems,
            *, T, FC, D, F):
    i = pl.program_id(0)
    nf = F // FC
    R = T // nf

    def cp_g(j):
        return pltpu.make_async_copy(wg_hbm.at[:, pl.ds(j * FC, FC)], wg_ref.at[j], sems.at[0, j])

    def cp_u(j):
        return pltpu.make_async_copy(wu_hbm.at[:, pl.ds(j * FC, FC)], wu_ref.at[j], sems.at[1, j])

    def cp_d(j):
        return pltpu.make_async_copy(wd_hbm.at[pl.ds(j * FC, FC), :], wd_ref.at[j], sems.at[2, j])

    def cp_qkv(m):
        return pltpu.make_async_copy(wqkv_hbm.at[:, pl.ds(m * D, D)], wqkv_ref.at[m], sems.at[3, m])

    cp_o = pltpu.make_async_copy(wo_hbm, wo_ref, sems.at[3, 3])

    @pl.when(i == 0)
    def _():
        cp_qkv(0).start()
        cp_qkv(1).start()
        acc_ref[...] = jnp.zeros(acc_ref.shape, jnp.float32)
        halo_scr[...] = jnp.zeros(halo_scr.shape, jnp.float32)

    def qkv_body(m, carry):
        @pl.when(i == 0)
        def _():
            cp_qkv(m).wait()

            @pl.when(m == 0)
            def _():
                cp_qkv(2).start()

            @pl.when(m == 1)
            def _():
                cp_g(0).start()
                cp_u(0).start()

            @pl.when(m == 2)
            def _():
                cp_d(0).start()

        y = jnp.dot(x_ref[...], wqkv_ref[m], preferred_element_type=jnp.float32)
        y = y.astype(jnp.bfloat16)
        ys = _swap_col_lane_bits([pltpu.bitcast(y[:, c * 128:(c + 1) * 128], jnp.uint32) for c in range(8)])
        for c in range(8):
            yc = pltpu.bitcast(ys[c], jnp.bfloat16).astype(jnp.float32)
            for s in range(nf):
                if s == 0:
                    qkv_scr[m, s, c, pl.ds(0, _HALO), :] = halo_scr[m, c]
                    qkv_scr[m, s, c, pl.ds(_HALO, R), :] = yc[0:R]
                else:
                    qkv_scr[m, s, c] = yc[s * R - _HALO:(s + 1) * R]
            halo_scr[m, c] = yc[T - _HALO:T]
        return carry
    jax.lax.fori_loop(0, 3, qkv_body, 0)

    scale = (D // _H) ** -0.5
    li = jax.lax.broadcasted_iota(jnp.int32, (128, 128), 0)
    lj = jax.lax.broadcasted_iota(jnp.int32, (128, 128), 1)
    E = jnp.where((li >> 2) == (lj >> 2), 1.0, 0.0).astype(jnp.bfloat16)

    def attn_strip(s):
        row = i * T + s * R + jax.lax.broadcasted_iota(jnp.int32, (R, 128), 0)
        q = [qkv_scr[0, s, c, pl.ds(_HALO, R), :] for c in range(8)]
        logits = []
        for w in range(_W):
            part = None
            for c in range(8):
                t = q[c] * qkv_scr[1, s, c, pl.ds(_HALO - _DIL * w, R), :]
                part = t if part is None else part + t
            l = jnp.dot(part.astype(jnp.bfloat16), E, preferred_element_type=jnp.float32) * scale
            if w > 0:
                l = jnp.where(row >= _DIL * w, l, -1e9)
            logits.append(l)
        mx = logits[0]
        for w in range(1, _W):
            mx = jnp.maximum(mx, logits[w])
        ps = [jnp.exp(l - mx) for l in logits]
        den = ps[0]
        for w in range(1, _W):
            den = den + ps[w]
        inv = 1.0 / den
        ps = [p * inv for p in ps]
        ocols = []
        for c in range(8):
            oc = None
            for w in range(_W):
                t = ps[w] * qkv_scr[2, s, c, pl.ds(_HALO - _DIL * w, R), :]
                oc = t if oc is None else oc + t
            ocols.append(pltpu.bitcast(oc.astype(jnp.bfloat16), jnp.uint32))
        ocols = _swap_col_lane_bits(ocols)
        for c in range(8):
            att_scr[s, :, pl.ds(c * 128, 128)] = pltpu.bitcast(ocols[c], jnp.bfloat16)

    def ffn_body(j, carry):
        @pl.when(i == 0)
        def _():
            cp_g(j).wait()
            cp_u(j).wait()
            cp_d(j).wait()

            @pl.when(j + 1 < nf)
            def _():
                cp_g(j + 1).start()
                cp_u(j + 1).start()
                cp_d(j + 1).start()

            @pl.when(j + 2 == nf)
            def _():
                cp_o.start()

        x = x_ref[...]
        gate = jnp.dot(x, wg_ref[j], preferred_element_type=jnp.float32)
        attn_strip(j)
        up = jnp.dot(x, wu_ref[j], preferred_element_type=jnp.float32)
        h = (jnp.where(gate > 0, gate, 0.0) * up).astype(jnp.bfloat16)
        acc_ref[...] += jnp.dot(h, wd_ref[j], preferred_element_type=jnp.float32)
        return carry
    jax.lax.fori_loop(0, nf, ffn_body, 0)

    @pl.when(i == 0)
    def _():
        cp_o.wait()

    a = jnp.dot(att_scr[...].reshape(T, D), wo_ref[...], preferred_element_type=jnp.float32)
    gl = jnp.sum(x_ref[...].astype(jnp.float32) * gw_ref[...].astype(jnp.float32), axis=-1, keepdims=True)
    g = jax.nn.sigmoid(gl)
    o_ref[...] = (g * a + (1.0 - g) * acc_ref[...]).astype(o_ref.dtype)
    acc_ref[...] = jnp.zeros(acc_ref.shape, jnp.float32)


@jax.jit
def pallas_gated_mix__sliding_local_dilated__glu_gated_reglu__prompt_kernel(
    A_x: jax.Array,
    A_wqkv: jax.Array,
    A_wo: jax.Array,
    B_x: jax.Array,
    B_W_gate: jax.Array,
    B_W_up: jax.Array,
    B_W_down: jax.Array,
    gate_w: jax.Array,
):
    del B_x
    B, S, D = A_x.shape
    F = B_W_gate.shape[1]
    T, FC = _T, _FC
    nf = F // FC
    x2 = A_x.reshape(B * S, D)
    gw2 = gate_w.reshape(1, D)
    any_spec = pl.BlockSpec(memory_space=pl.ANY)
    out = pl.pallas_call(
        functools.partial(_kernel, T=T, FC=FC, D=D, F=F),
        grid=(S // T,),
        in_specs=[
            pl.BlockSpec((T, D), lambda i: (i, 0)),
            pl.BlockSpec((1, D), lambda i: (0, 0)),
            any_spec, any_spec, any_spec, any_spec, any_spec,
        ],
        out_specs=pl.BlockSpec((T, D), lambda i: (i, 0)),
        out_shape=jax.ShapeDtypeStruct((B * S, D), A_x.dtype),
        scratch_shapes=[
            pltpu.VMEM((3, D, D), jnp.bfloat16),
            pltpu.VMEM((D, D), jnp.bfloat16),
            pltpu.VMEM((nf, D, FC), jnp.bfloat16),
            pltpu.VMEM((nf, D, FC), jnp.bfloat16),
            pltpu.VMEM((nf, FC, D), jnp.bfloat16),
            pltpu.VMEM((3, nf, 8, T // nf + _HALO, 128), jnp.float32),
            pltpu.VMEM((3, 8, _HALO, 128), jnp.float32),
            pltpu.VMEM((nf, T // nf, D), jnp.bfloat16),
            pltpu.VMEM((T, D), jnp.float32),
            pltpu.SemaphoreType.DMA((4, max(nf, 4))),
        ],
        compiler_params=pltpu.CompilerParams(
            dimension_semantics=("arbitrary",),
            vmem_limit_bytes=100 * 1024 * 1024,
        ),
    )(x2, gw2, A_wqkv, A_wo, B_W_gate, B_W_up, B_W_down)
    return out.reshape(B, S, D)
```

```python
import functools

import jax
import jax.numpy as jnp
import jax.experimental.pallas as pl
import jax.experimental.pallas.tpu as pltpu

_H = 32
_W = 8
_DIL = 2
_HALO = 16

_T = 512
_FC = 896


def _swap_col_lane_bits(cols):
    lane = jax.lax.broadcasted_iota(jnp.int32, cols[0].shape, 1)
    cols = list(cols)
    for b in range(3):
        s = 4 << b
        hi = (lane & s) != 0
        new = list(cols)
        for a in range(8):
            if a & (1 << b):
                continue
            A, B = cols[a], cols[a | (1 << b)]
            new[a] = jnp.where(hi, pltpu.roll(B, s, 1), A)
            new[a | (1 << b)] = jnp.where(hi, B, pltpu.roll(A, 128 - s, 1))
        cols = new
    return cols


def _kernel(x_ref, gw_ref, wqkv_hbm, wo_hbm, wg_hbm, wu_hbm, wd_hbm, o_ref,
            wqkv_ref, wo_ref, wg_ref, wu_ref, wd_ref, qkv_scr, halo_scr, att_scr, acc_ref, sems,
            *, T, FC, D, F):
    i = pl.program_id(0)
    nf = F // FC
    R = T // nf

    def cp_g(j):
        return pltpu.make_async_copy(wg_hbm.at[:, pl.ds(j * FC, FC)], wg_ref.at[j], sems.at[0, j])

    def cp_u(j):
        return pltpu.make_async_copy(wu_hbm.at[:, pl.ds(j * FC, FC)], wu_ref.at[j], sems.at[1, j])

    def cp_d(j):
        return pltpu.make_async_copy(wd_hbm.at[pl.ds(j * FC, FC), :], wd_ref.at[j], sems.at[2, j])

    def cp_qkv(m):
        return pltpu.make_async_copy(wqkv_hbm.at[:, pl.ds(m * D, D)], wqkv_ref.at[m], sems.at[3, m])

    cp_o = pltpu.make_async_copy(wo_hbm, wo_ref, sems.at[3, 3])

    @pl.when(i == 0)
    def _():
        cp_qkv(0).start()
        cp_qkv(1).start()
        acc_ref[...] = jnp.zeros(acc_ref.shape, jnp.float32)
        halo_scr[...] = jnp.zeros(halo_scr.shape, jnp.float32)

    def qkv_body(m, carry):
        @pl.when(i == 0)
        def _():
            cp_qkv(m).wait()

            @pl.when(m == 0)
            def _():
                cp_qkv(2).start()

            @pl.when(m == 1)
            def _():
                cp_g(0).start()
                cp_u(0).start()

            @pl.when(m == 2)
            def _():
                cp_d(0).start()

        y = jnp.dot(x_ref[...], wqkv_ref[m], preferred_element_type=jnp.float32)
        y = y.astype(jnp.bfloat16)
        ys = _swap_col_lane_bits([pltpu.bitcast(y[:, c * 128:(c + 1) * 128], jnp.uint32) for c in range(8)])
        for c in range(8):
            yc = pltpu.bitcast(ys[c], jnp.bfloat16).astype(jnp.float32)
            for s in range(nf):
                if s == 0:
                    qkv_scr[m, s, c, pl.ds(0, _HALO), :] = halo_scr[m, c]
                    qkv_scr[m, s, c, pl.ds(_HALO, R), :] = yc[0:R]
                else:
                    qkv_scr[m, s, c] = yc[s * R - _HALO:(s + 1) * R]
            halo_scr[m, c] = yc[T - _HALO:T]
        return carry
    jax.lax.fori_loop(0, 3, qkv_body, 0, unroll=True)

    scale = (D // _H) ** -0.5
    def attn_strip(s):
        row = i * T + s * R + jax.lax.broadcasted_iota(jnp.int32, (R, 128), 0)
        lane = jax.lax.broadcasted_iota(jnp.int32, (R, 128), 1)
        q = [qkv_scr[0, s, c, pl.ds(_HALO, R), :] for c in range(8)]
        logits = []
        for w in range(_W):
            part = None
            for c in range(8):
                t = q[c] * qkv_scr[1, s, c, pl.ds(_HALO - _DIL * w, R), :]
                part = t if part is None else part + t
            for b in (1, 2):
                part = part + jnp.where((lane & b) != 0, pltpu.roll(part, b, 1), pltpu.roll(part, 128 - b, 1))
            l = part * scale
            if w > 0:
                l = jnp.where(row >= _DIL * w, l, -1e9)
            logits.append(l)
        mx = logits[0]
        for w in range(1, _W):
            mx = jnp.maximum(mx, logits[w])
        ps = [jnp.exp(l - mx) for l in logits]
        den = ps[0]
        for w in range(1, _W):
            den = den + ps[w]
        inv = 1.0 / den
        ps = [p * inv for p in ps]
        ocols = []
        for c in range(8):
            oc = None
            for w in range(_W):
                t = ps[w] * qkv_scr[2, s, c, pl.ds(_HALO - _DIL * w, R), :]
                oc = t if oc is None else oc + t
            ocols.append(pltpu.bitcast(oc.astype(jnp.bfloat16), jnp.uint32))
        ocols = _swap_col_lane_bits(ocols)
        for c in range(8):
            att_scr[s, :, pl.ds(c * 128, 128)] = pltpu.bitcast(ocols[c], jnp.bfloat16)

    def ffn_body(j, carry):
        @pl.when(i == 0)
        def _():
            cp_g(j).wait()
            cp_u(j).wait()
            cp_d(j).wait()

            @pl.when(j + 1 < nf)
            def _():
                cp_g(j + 1).start()
                cp_u(j + 1).start()
                cp_d(j + 1).start()

            @pl.when(j + 2 == nf)
            def _():
                cp_o.start()

        x = x_ref[...]
        gate = jnp.dot(x, wg_ref[j], preferred_element_type=jnp.float32)
        attn_strip(j)
        up = jnp.dot(x, wu_ref[j], preferred_element_type=jnp.float32)
        h = (jnp.where(gate > 0, gate, 0.0) * up).astype(jnp.bfloat16)
        acc_ref[...] += jnp.dot(h, wd_ref[j], preferred_element_type=jnp.float32)
        return carry
    jax.lax.fori_loop(0, nf, ffn_body, 0)

    @pl.when(i == 0)
    def _():
        cp_o.wait()

    a = jnp.dot(att_scr[...].reshape(T, D), wo_ref[...], preferred_element_type=jnp.float32)
    gl = jnp.sum(x_ref[...].astype(jnp.float32) * gw_ref[...].astype(jnp.float32), axis=-1, keepdims=True)
    g = jax.nn.sigmoid(gl)
    o_ref[...] = (g * a + (1.0 - g) * acc_ref[...]).astype(o_ref.dtype)
    acc_ref[...] = jnp.zeros(acc_ref.shape, jnp.float32)


@jax.jit
def pallas_gated_mix__sliding_local_dilated__glu_gated_reglu__prompt_kernel(
    A_x: jax.Array,
    A_wqkv: jax.Array,
    A_wo: jax.Array,
    B_x: jax.Array,
    B_W_gate: jax.Array,
    B_W_up: jax.Array,
    B_W_down: jax.Array,
    gate_w: jax.Array,
):
    del B_x
    B, S, D = A_x.shape
    F = B_W_gate.shape[1]
    T, FC = _T, _FC
    nf = F // FC
    x2 = A_x.reshape(B * S, D)
    gw2 = gate_w.reshape(1, D)
    any_spec = pl.BlockSpec(memory_space=pl.ANY)
    out = pl.pallas_call(
        functools.partial(_kernel, T=T, FC=FC, D=D, F=F),
        grid=(S // T,),
        in_specs=[
            pl.BlockSpec((T, D), lambda i: (i, 0)),
            pl.BlockSpec((1, D), lambda i: (0, 0)),
            any_spec, any_spec, any_spec, any_spec, any_spec,
        ],
        out_specs=pl.BlockSpec((T, D), lambda i: (i, 0)),
        out_shape=jax.ShapeDtypeStruct((B * S, D), A_x.dtype),
        scratch_shapes=[
            pltpu.VMEM((3, D, D), jnp.bfloat16),
            pltpu.VMEM((D, D), jnp.bfloat16),
            pltpu.VMEM((nf, D, FC), jnp.bfloat16),
            pltpu.VMEM((nf, D, FC), jnp.bfloat16),
            pltpu.VMEM((nf, FC, D), jnp.bfloat16),
            pltpu.VMEM((3, nf, 8, T // nf + _HALO, 128), jnp.float32),
            pltpu.VMEM((3, 8, _HALO, 128), jnp.float32),
            pltpu.VMEM((nf, T // nf, D), jnp.bfloat16),
            pltpu.VMEM((T, D), jnp.float32),
            pltpu.SemaphoreType.DMA((4, max(nf, 4))),
        ],
        compiler_params=pltpu.CompilerParams(
            dimension_semantics=("arbitrary",),
            vmem_limit_bytes=100 * 1024 * 1024,
        ),
    )(x2, gw2, A_wqkv, A_wo, B_W_gate, B_W_up, B_W_down)
    return out.reshape(B, S, D)
```

```python
import functools

import jax
import jax.numpy as jnp
import jax.experimental.pallas as pl
import jax.experimental.pallas.tpu as pltpu

_H = 32
_W = 8
_DIL = 2
_HALO = 16

_T = 512
_FC = 896


def _swap_col_lane_bits(cols):
    lane = jax.lax.broadcasted_iota(jnp.int32, cols[0].shape, 1)
    cols = list(cols)
    for b in range(3):
        s = 4 << b
        hi = (lane & s) != 0
        new = list(cols)
        for a in range(8):
            if a & (1 << b):
                continue
            A, B = cols[a], cols[a | (1 << b)]
            new[a] = jnp.where(hi, pltpu.roll(B, s, 1), A)
            new[a | (1 << b)] = jnp.where(hi, B, pltpu.roll(A, 128 - s, 1))
        cols = new
    return cols


def _kernel(x_ref, gw_ref, wqkv_hbm, wo_hbm, wg_hbm, wu_hbm, wd_hbm, o_ref,
            wqkv_ref, wo_ref, wg_ref, wu_ref, wd_ref, qkv_scr, halo_scr, att_scr, acc_ref, sems,
            *, T, FC, D, F):
    i = pl.program_id(0)
    nf = F // FC
    R = T // nf

    def cp_g(j):
        return pltpu.make_async_copy(wg_hbm.at[:, pl.ds(j * FC, FC)], wg_ref.at[j], sems.at[0, j])

    def cp_u(j):
        return pltpu.make_async_copy(wu_hbm.at[:, pl.ds(j * FC, FC)], wu_ref.at[j], sems.at[1, j])

    def cp_d(j):
        return pltpu.make_async_copy(wd_hbm.at[pl.ds(j * FC, FC), :], wd_ref.at[j], sems.at[2, j])

    def cp_qkv(m):
        return pltpu.make_async_copy(wqkv_hbm.at[:, pl.ds(m * D, D)], wqkv_ref.at[m], sems.at[3, m])

    cp_o = pltpu.make_async_copy(wo_hbm, wo_ref, sems.at[3, 3])

    @pl.when(i == 0)
    def _():
        cp_qkv(0).start()
        cp_qkv(1).start()
        acc_ref[...] = jnp.zeros(acc_ref.shape, jnp.float32)
        halo_scr[...] = jnp.zeros(halo_scr.shape, jnp.float32)

    def qkv_mm(m):
        @pl.when(i == 0)
        def _():
            cp_qkv(m).wait()

            @pl.when(bool(m == 0))
            def _():
                cp_qkv(2).start()

            @pl.when(bool(m == 1))
            def _():
                cp_g(0).start()
                cp_u(0).start()

            @pl.when(bool(m == 2))
            def _():
                cp_d(0).start()

        y = jnp.dot(x_ref[...], wqkv_ref[m], preferred_element_type=jnp.float32)
        return y.astype(jnp.bfloat16)

    def qkv_post(m, y):
        ys = _swap_col_lane_bits([pltpu.bitcast(y[:, c * 128:(c + 1) * 128], jnp.uint32) for c in range(8)])
        for c in range(8):
            yc = pltpu.bitcast(ys[c], jnp.bfloat16).astype(jnp.float32)
            for s in range(nf):
                if s == 0:
                    qkv_scr[m, s, c, pl.ds(0, _HALO), :] = halo_scr[m, c]
                    qkv_scr[m, s, c, pl.ds(_HALO, R), :] = yc[0:R]
                else:
                    qkv_scr[m, s, c] = yc[s * R - _HALO:(s + 1) * R]
            halo_scr[m, c] = yc[T - _HALO:T]

    yq = qkv_mm(0)
    yk = qkv_mm(1)
    qkv_post(0, yq)
    yv = qkv_mm(2)
    qkv_post(1, yk)
    qkv_post(2, yv)

    scale = (D // _H) ** -0.5
    def attn_strip(s):
        row = i * T + s * R + jax.lax.broadcasted_iota(jnp.int32, (R, 128), 0)
        lane = jax.lax.broadcasted_iota(jnp.int32, (R, 128), 1)
        q = [qkv_scr[0, s, c, pl.ds(_HALO, R), :] for c in range(8)]
        logits = []
        for w in range(_W):
            part = None
            for c in range(8):
                t = q[c] * qkv_scr[1, s, c, pl.ds(_HALO - _DIL * w, R), :]
                part = t if part is None else part + t
            for b in (1, 2):
                part = part + jnp.where((lane & b) != 0, pltpu.roll(part, b, 1), pltpu.roll(part, 128 - b, 1))
            l = part * scale
            if w > 0:
                l = jnp.where(row >= _DIL * w, l, -1e9)
            logits.append(l)
        mx = logits[0]
        for w in range(1, _W):
            mx = jnp.maximum(mx, logits[w])
        ps = [jnp.exp(l - mx) for l in logits]
        den = ps[0]
        for w in range(1, _W):
            den = den + ps[w]
        inv = 1.0 / den
        ps = [p * inv for p in ps]
        ocols = []
        for c in range(8):
            oc = None
            for w in range(_W):
                t = ps[w] * qkv_scr[2, s, c, pl.ds(_HALO - _DIL * w, R), :]
                oc = t if oc is None else oc + t
            ocols.append(pltpu.bitcast(oc.astype(jnp.bfloat16), jnp.uint32))
        ocols = _swap_col_lane_bits(ocols)
        for c in range(8):
            att_scr[s, :, pl.ds(c * 128, 128)] = pltpu.bitcast(ocols[c], jnp.bfloat16)

    def ffn_body(j, carry):
        @pl.when(i == 0)
        def _():
            cp_g(j).wait()
            cp_u(j).wait()
            cp_d(j).wait()

            @pl.when(j + 1 < nf)
            def _():
                cp_g(j + 1).start()
                cp_u(j + 1).start()
                cp_d(j + 1).start()

            @pl.when(j + 2 == nf)
            def _():
                cp_o.start()

        x = x_ref[...]
        gate = jnp.dot(x, wg_ref[j], preferred_element_type=jnp.float32)
        attn_strip(j)
        up = jnp.dot(x, wu_ref[j], preferred_element_type=jnp.float32)
        h = (jnp.where(gate > 0, gate, 0.0) * up).astype(jnp.bfloat16)
        acc_ref[...] += jnp.dot(h, wd_ref[j], preferred_element_type=jnp.float32)
        return carry
    jax.lax.fori_loop(0, nf, ffn_body, 0)

    @pl.when(i == 0)
    def _():
        cp_o.wait()

    a = jnp.dot(att_scr[...].reshape(T, D), wo_ref[...], preferred_element_type=jnp.float32)
    gl = jnp.sum(x_ref[...].astype(jnp.float32) * gw_ref[...].astype(jnp.float32), axis=-1, keepdims=True)
    g = jax.nn.sigmoid(gl)
    o_ref[...] = (g * a + (1.0 - g) * acc_ref[...]).astype(o_ref.dtype)
    acc_ref[...] = jnp.zeros(acc_ref.shape, jnp.float32)


@jax.jit
def pallas_gated_mix__sliding_local_dilated__glu_gated_reglu__prompt_kernel(
    A_x: jax.Array,
    A_wqkv: jax.Array,
    A_wo: jax.Array,
    B_x: jax.Array,
    B_W_gate: jax.Array,
    B_W_up: jax.Array,
    B_W_down: jax.Array,
    gate_w: jax.Array,
):
    del B_x
    B, S, D = A_x.shape
    F = B_W_gate.shape[1]
    T, FC = _T, _FC
    nf = F // FC
    x2 = A_x.reshape(B * S, D)
    gw2 = gate_w.reshape(1, D)
    any_spec = pl.BlockSpec(memory_space=pl.ANY)
    out = pl.pallas_call(
        functools.partial(_kernel, T=T, FC=FC, D=D, F=F),
        grid=(S // T,),
        in_specs=[
            pl.BlockSpec((T, D), lambda i: (i, 0)),
            pl.BlockSpec((1, D), lambda i: (0, 0)),
            any_spec, any_spec, any_spec, any_spec, any_spec,
        ],
        out_specs=pl.BlockSpec((T, D), lambda i: (i, 0)),
        out_shape=jax.ShapeDtypeStruct((B * S, D), A_x.dtype),
        scratch_shapes=[
            pltpu.VMEM((3, D, D), jnp.bfloat16),
            pltpu.VMEM((D, D), jnp.bfloat16),
            pltpu.VMEM((nf, D, FC), jnp.bfloat16),
            pltpu.VMEM((nf, D, FC), jnp.bfloat16),
            pltpu.VMEM((nf, FC, D), jnp.bfloat16),
            pltpu.VMEM((3, nf, 8, T // nf + _HALO, 128), jnp.float32),
            pltpu.VMEM((3, 8, _HALO, 128), jnp.float32),
            pltpu.VMEM((nf, T // nf, D), jnp.bfloat16),
            pltpu.VMEM((T, D), jnp.float32),
            pltpu.SemaphoreType.DMA((4, max(nf, 4))),
        ],
        compiler_params=pltpu.CompilerParams(
            dimension_semantics=("arbitrary",),
            vmem_limit_bytes=100 * 1024 * 1024,
        ),
    )(x2, gw2, A_wqkv, A_wo, B_W_gate, B_W_up, B_W_down)
    return out.reshape(B, S, D)
```
